```python
import jax
import jax.numpy as jnp

def _softmax(x, axis=-1):
    return jax.nn.softmax(x, axis=axis)

def _gelu(x):
    return jax.nn.gelu(x, approximate=True)

def _silu(x):
    return jax.nn.silu(x)

def _sigmoid(x):
    return jax.nn.sigmoid(x)

def _layernorm(x, axis=-1, eps=1e-05):
    m = jnp.mean(x, axis=axis, keepdims=True)
    v = jnp.var(x, axis=axis, keepdims=True)
    return (x - m) / jnp.sqrt(v + eps)

def _scatter_add(tgt, idx, src, axis=0):
    return tgt.at[idx].add(src)

def _segment_sum(src, seg, n):
    return jax.ops.segment_sum(src, seg, n)

class _Rng:

    def __init__(self, key):
        self._k = key

    def _next(self):
        self._k, sub = jax.random.split(self._k)
        return sub

    def normal(self, shape):
        return jax.random.normal(self._next(), shape, dtype=jnp.bfloat16)

    def randint(self, lo, hi, shape):
        return jax.random.randint(self._next(), shape, lo, hi, dtype=jnp.int32)

    def uniform(self, shape, lo=0.0, hi=1.0):
        return jax.random.uniform(self._next(), shape, jnp.bfloat16, lo, hi)

    def permutation(self, n):
        return jax.random.permutation(self._next(), n)
kernel_name = 'sequential_preLN__memory_aug_recurrent_mem_tr__mixer_s_mlp__prompt'

def setup_inputs():
    _rng = _Rng(jax.random.key(int.from_bytes(__import__("os").urandom(4), "little")))
    _w = lambda a: (lambda t: t.astype(jnp.bfloat16) if jnp.issubdtype(t.dtype, jnp.floating) else t)(jnp.asarray(a))

    def _A_setup():
        B, S, Dm = (1, 2048, 1024)
        H, Dh = (32, 128)
        M, seg = (8, 32)
        seg = min(seg, S)
        S = S // seg * seg
        return {'x': _w((lambda *s: _rng.normal(s) * 0.05)(B, S, Dm)), 'mem0': _w((lambda *s: _rng.normal(s) * 0.05)(B, M, Dm)), 'Wq': _w((lambda *s: _rng.normal(s) * 0.05)(Dm, H, Dh) * Dm ** (-0.5)), 'Wk': _w((lambda *s: _rng.normal(s) * 0.05)(Dm, H, Dh) * Dm ** (-0.5)), 'Wv': _w((lambda *s: _rng.normal(s) * 0.05)(Dm, H, Dh) * Dm ** (-0.5)), 'Wo': _w((lambda *s: _rng.normal(s) * 0.05)(H, Dh, Dm) * (H * Dh) ** (-0.5)), 'seg_len': seg}
    _A_in = _A_setup()

    def _B_setup():
        B, S, D, F = (1, 2048, 1024, 3584)
        return {'x': _w((lambda *s: _rng.normal(s) * 0.05)(B, S, D)), 'w1': _w((lambda *s: _rng.normal(s) * 0.05)(D, D) * D ** (-0.5)), 'w2': _w((lambda *s: _rng.normal(s) * 0.05)(D, D) * D ** (-0.5)), 'w3': _w((lambda *s: _rng.normal(s) * 0.05)(D, F) * D ** (-0.5)), 'w4': _w((lambda *s: _rng.normal(s) * 0.05)(F, D) * F ** (-0.5))}
    _B_in = _B_setup()
    return {'A_x': _A_in['x'], 'A_mem0': _A_in['mem0'], 'A_Wq': _A_in['Wq'], 'A_Wk': _A_in['Wk'], 'A_Wv': _A_in['Wv'], 'A_Wo': _A_in['Wo'], 'A_seg_len': _A_in['seg_len'], 'B_x': _B_in['x'], 'B_w1': _B_in['w1'], 'B_w2': _B_in['w2'], 'B_w3': _B_in['w3'], 'B_w4': _B_in['w4']}

def reference(A_x, A_mem0, A_Wq, A_Wk, A_Wv, A_Wo, A_seg_len, B_x, B_w1, B_w2, B_w3, B_w4):

    def _A_ref(x, mem0, Wq, Wk, Wv, Wo, seg_len):
        B, S, Dm = x.shape
        H, Dh = (Wq.shape[1], Wq.shape[2])
        M = mem0.shape[1]
        scale = Dh ** (-0.5)
        n_seg = S // seg_len
        L = M + seg_len
        idx = jnp.arange(L)
        mask = (idx[:, None] < M) | (idx[:, None] >= idx[None, :])
        mem = mem0
        outs = []
        for s in range(n_seg):
            xs = x[:, s * seg_len:(s + 1) * seg_len, :].copy()
            h = jnp.concatenate([mem, xs], axis=1)
            q = jnp.einsum('btd,dhe->bhte', h, Wq)
            k = jnp.einsum('btd,dhe->bhte', h, Wk)
            v = jnp.einsum('btd,dhe->bhte', h, Wv)
            scores = jnp.einsum('bhqe,bhke->bhqk', q, k) * scale
            scores = jnp.where(mask[None, None], scores, -1000000000.0)
            p = _softmax(scores, axis=-1)
            o = jnp.einsum('bhqk,bhke->bhqe', p, v)
            o = jnp.einsum('bhte,hed->btd', o, Wo)
            mem = o[:, :M, :].copy()
            outs.append(o[:, M:, :])
        return jnp.concatenate(outs, axis=1)

    def _B_ref(x, w1, w2, w3, w4):
        B, S, D = x.shape
        h = _gelu(_layernorm(x, axis=-1) @ w1)
        c = D // 4
        g0 = jnp.pad(h[:, :, 0 * c:1 * c], ((0, 0), (1, 0), (0, 0)))[:, :S, :]
        g1 = jnp.pad(h[:, :, 1 * c:2 * c], ((0, 0), (0, 1), (0, 0)))[:, 1:, :]
        g2 = jnp.pad(h[:, :, 2 * c:3 * c], ((0, 0), (2, 0), (0, 0)))[:, :S, :]
        g3 = jnp.pad(h[:, :, 3 * c:], ((0, 0), (0, 2), (0, 0)))[:, 2:, :]
        hs = jnp.concatenate([g0, g1, g2, g3], axis=-1) @ w2
        x1 = x + hs
        h2 = _gelu(_layernorm(x1, axis=-1) @ w3) @ w4
        return x1 + h2
    x = A_x
    h = x + _A_ref(_layernorm(x, axis=-1), A_mem0, A_Wq, A_Wk, A_Wv, A_Wo, A_seg_len)
    h2 = h + _B_ref(_layernorm(h, axis=-1), B_w1, B_w2, B_w3, B_w4)
    return h2
```

```python
import functools

import jax
import jax.numpy as jnp
import numpy as np
from jax import lax
from jax.experimental import pallas as pl
from jax.experimental.pallas import tpu as pltpu

F32 = jnp.float32
BF16 = jnp.bfloat16
U32 = jnp.uint32


def _ln(x):
    m = jnp.mean(x, axis=-1, keepdims=True)
    xc = x - m
    v = jnp.mean(xc * xc, axis=-1, keepdims=True)
    return xc * lax.rsqrt(v + 1e-5)


def _gelu(x):
    c = 0.7978845608028654
    return 0.5 * x * (1.0 + jnp.tanh(c * (x + 0.044715 * (x * x * x))))


def _mm(a, b):
    return lax.dot_general(a, b, (((1,), (0,)), ((), ())), preferred_element_type=F32)


def _mm_nt(a, b):
    return lax.dot_general(a, b, (((1,), (1,)), ((), ())), preferred_element_type=F32)


def build(S, D, H, E, M, SEG, F, *, G=4, RB=256, DELAY_O=False, name="k1"):
    NSEG = S // SEG
    L = M + SEG
    scale = float(E) ** -0.5
    NB = S // RB
    HP = H // 2

    def kernel(x_hbm, mem0_ref, wq_hbm, wk_hbm, wv_hbm, wo_hbm, w1_hbm, w2_hbm, w3_hbm, w4_hbm,
               out_hbm,
               x_v, hbuf, stage, wq_s, wk_s, wv_s, wo_s, w1_s, w2_s, w3_s, w4_s, t_s, ob, sems, osem):
        cp_x = pltpu.make_async_copy(x_hbm, x_v, sems.at[0])
        cp_x.start()
        cp_w = []
        for i, w in enumerate((wq_hbm, wk_hbm, wv_hbm)):
            c = pltpu.make_async_copy(w.bitcast(U32), stage.at[i], sems.at[1 + i])
            c.start()
            cp_w.append(c)
        cp_o = []
        for j in range(D // 128):
            c = pltpu.make_async_copy(wo_hbm.at[:, pl.ds(j * 128, 128)], wo_s.at[j], sems.at[4 + j])
            c.start()
            cp_o.append(c)
        cp_b = []
        for i, (src, dst) in enumerate(((w1_hbm, w1_s), (w2_hbm, w2_s), (w3_hbm, w3_s), (w4_hbm, w4_s))):
            c = pltpu.make_async_copy(src, dst, sems.at[12 + i])
            c.start()
            cp_b.append(c)

        cp_x.wait()

        def ln_body(i, c):
            r = pl.ds(pl.multiple_of(i * 256, 256), 256)
            hbuf[r, :] = _ln(x_v[r, :].astype(F32)).astype(BF16).astype(F32)
            return c
        lax.fori_loop(0, S // 256, ln_body, 0)

        for i, dst in enumerate((wq_s, wk_s, wv_s)):
            cp_w[i].wait()

            def rl_body(p, c, i=i, dst=dst):
                a = stage[i, pl.ds(p, D // 2, stride=2 * HP), :]
                b = stage[i, pl.ds(HP + p, D // 2, stride=2 * HP), :]
                dst[2 * p] = (a & 0xFFFF) | (b << 16)
                dst[2 * p + 1] = (a >> 16) | (b & np.uint32(0xFFFF0000))
                return c
            lax.fori_loop(0, HP, rl_body, 0)
        for c in cp_o:
            c.wait()

        def wcat(ref, h0, n):
            return jnp.concatenate([pltpu.bitcast(ref[h], BF16) for h in range(h0, h0 + n)], axis=1)

        def step(s, mem):
            r = pl.ds(pl.multiple_of(s * SEG, SEG), SEG)
            xs = hbuf[r, :]
            hs = jnp.concatenate([mem, xs], axis=0)
            row = lax.broadcasted_iota(jnp.int32, (L, 128), 0)
            col = lax.broadcasted_iota(jnp.int32, (L, 128), 1)
            mask = ((row < M) | (row >= col)) & (col < L)
            zpad = jnp.zeros((8, E), F32)
            zpad2 = jnp.zeros((128 - 48, E), BF16)
            NG = H // G

            def proj(ref, g):
                return _mm(hs, wcat(ref, g * G, G))

            def pad_kv(t):
                return jnp.concatenate([jnp.concatenate([t, zpad], axis=0).astype(BF16), zpad2], axis=0)

            def qk(q, k):
                out = []
                for j in range(G):
                    sl = slice(j * E, (j + 1) * E)
                    out.append(_mm_nt(q[:, sl], pad_kv(k[:, sl])))
                return out

            def soft(scs):
                out = []
                for sc in scs:
                    sc = jnp.where(mask, sc * scale, -1e9)
                    mx = jnp.max(sc, axis=-1, keepdims=True)
                    p = jnp.exp(sc - mx)
                    out.append((p, jnp.sum(p, axis=-1, keepdims=True)))
                return out

            def pv(ps, v):
                out = []
                for j in range(G):
                    sl = slice(j * E, (j + 1) * E)
                    out.append(_mm(ps[j][0], pad_kv(v[:, sl])) * (1.0 / ps[j][1]))
                return jnp.concatenate(out, axis=1)

            def oproj(og, g):
                wo = jnp.concatenate([wo_s[j, pl.ds(g * G * E, G * E), :] for j in range(D // 128)], axis=1)
                return _mm(og, wo)

            acc = None
            q, k, v = proj(wq_s, 0), proj(wk_s, 0), proj(wv_s, 0)
            pend = None
            for g in range(NG):
                last = g == NG - 1
                if not last:
                    q2 = proj(wq_s, g + 1)
                scs = qk(q, k)
                if not last:
                    k2 = proj(wk_s, g + 1)
                else:
                    acc = acc + oproj(*pend)
                og = pv(soft(scs), v)
                if not last:
                    v2 = proj(wv_s, g + 1)
                if DELAY_O:
                    if pend is not None and not last:
                        y = oproj(*pend)
                        acc = y if acc is None else acc + y
                    pend = (og, g)
                else:
                    if g == NG - 2:
                        pend = (og, g)
                    else:
                        y = oproj(og, g)
                        acc = y if acc is None else acc + y
                if not last:
                    q, k, v = q2, k2, v2
            if DELAY_O:
                acc = acc + oproj(*pend)
            hbuf[r, :] = x_v[r, :].astype(F32) + acc[M:, :]
            return acc[:M, :]

        lax.fori_loop(0, NSEG, step, mem0_ref[...].astype(F32))

        for c in cp_b:
            c.wait()
        t_s[pl.ds(0, 8), :] = jnp.zeros((8, D), F32)
        t_s[pl.ds(8 + S, 8), :] = jnp.zeros((8, D), F32)

        def b1(i, c):
            r0 = pl.multiple_of(i * RB, RB)
            hn = _ln(hbuf[pl.ds(r0, RB), :])
            t_s[pl.ds(r0 + 8, RB), :] = _gelu(_mm(_ln(hn), w1_s[...]))
            return c
        lax.fori_loop(0, NB, b1, 0)

        C = D // 4

        def out_copy(i, slot):
            return pltpu.make_async_copy(ob.at[slot], out_hbm.at[pl.ds(pl.multiple_of(i * RB, RB), RB), :],
                                         osem.at[slot])

        def b2(i, c):
            r0 = pl.multiple_of(i * RB, RB)
            h = hbuf[pl.ds(r0, RB), :]
            hn = _ln(h)
            te = t_s[pl.ds(r0, RB + 16), :]
            n = RB + 16
            g0 = pltpu.roll(te[:, 0 * C:1 * C], 1, 0)
            g1 = pltpu.roll(te[:, 1 * C:2 * C], n - 1, 0)
            g2 = pltpu.roll(te[:, 2 * C:3 * C], 2, 0)
            g3 = pltpu.roll(te[:, 3 * C:4 * C], n - 2, 0)
            gs = jnp.concatenate([g0, g1, g2, g3], axis=1)[8:8 + RB, :]
            x1 = hn + _mm(gs, w2_s[...])
            u = _gelu(_mm(_ln(x1), w3_s[...]))
            res = h + x1 + _mm(u, w4_s[...])
            slot = i % 2

            @pl.when(i >= 2)
            def _():
                out_copy(i - 2, slot).wait()
            ob[slot] = res.astype(BF16)
            out_copy(i, slot).start()
            return c
        lax.fori_loop(0, NB, b2, 0)
        out_copy(NB - 2, 0).wait()
        out_copy(NB - 1, 1).wait()

    any_spec = pl.BlockSpec(memory_space=pl.ANY)
    vmem = pl.BlockSpec(memory_space=pltpu.VMEM)
    call = pl.pallas_call(
        kernel,
        out_shape=jax.ShapeDtypeStruct((S, D), BF16),
        in_specs=[any_spec, vmem] + [any_spec] * 8,
        out_specs=any_spec,
        scratch_shapes=[
            pltpu.VMEM((S, D), BF16),
            pltpu.VMEM((S, D), F32),
            pltpu.VMEM((3, D * HP, E), U32),
            pltpu.VMEM((H, D // 2, E), U32),
            pltpu.VMEM((H, D // 2, E), U32),
            pltpu.VMEM((H, D // 2, E), U32),
            pltpu.VMEM((D // 128, H * E, 128), BF16),
            pltpu.VMEM((D, D), BF16),
            pltpu.VMEM((D, D), BF16),
            pltpu.VMEM((D, F), BF16),
            pltpu.VMEM((F, D), BF16),
            pltpu.VMEM((S + 16, D), F32),
            pltpu.VMEM((2, RB, D), BF16),
            pltpu.SemaphoreType.DMA((16,)),
            pltpu.SemaphoreType.DMA((2,)),
        ],
        compiler_params=pltpu.CompilerParams(vmem_limit_bytes=120 * 2**20),
        name=name,
    )

    def run(A_x, A_mem0, A_Wq, A_Wk, A_Wv, A_Wo, B_w1, B_w2, B_w3, B_w4):
        out = call(A_x.reshape(S, D), A_mem0.reshape(M, D), A_Wq.reshape(D * H, E), A_Wk.reshape(D * H, E),
                   A_Wv.reshape(D * H, E), A_Wo.reshape(H * E, D), B_w1, B_w2, B_w3, B_w4)
        return out.reshape(1, S, D)
    return run


@functools.partial(jax.jit, static_argnames=("A_seg_len",))
def pallas_sequential_preLN__memory_aug_recurrent_mem_tr__mixer_s_mlp__prompt_kernel(
        A_x, A_mem0, A_Wq, A_Wk, A_Wv, A_Wo, A_seg_len, B_x, B_w1, B_w2, B_w3, B_w4):
    del B_x
    _, S, D = A_x.shape
    M = A_mem0.shape[1]
    H, E = A_Wq.shape[1], A_Wq.shape[2]
    F = B_w3.shape[1]
    run = build(S, D, H, E, M, int(A_seg_len), F)
    return run(A_x, A_mem0, A_Wq, A_Wk, A_Wv, A_Wo, B_w1, B_w2, B_w3, B_w4)
```

```python
import contextlib
import functools

import jax
import jax.numpy as jnp
import numpy as np
from jax import lax
from jax.experimental import pallas as pl
from jax.experimental.pallas import tpu as pltpu

F32 = jnp.float32
BF16 = jnp.bfloat16
U32 = jnp.uint32


def _ln(x):
    m = jnp.mean(x, axis=-1, keepdims=True)
    xc = x - m
    v = jnp.mean(xc * xc, axis=-1, keepdims=True)
    return xc * lax.rsqrt(v + 1e-5)


def _gelu(x):
    c = 0.7978845608028654
    return 0.5 * x * (1.0 + jnp.tanh(c * (x + 0.044715 * (x * x * x))))


def _mm(a, b):
    return lax.dot_general(a, b, (((1,), (0,)), ((), ())), preferred_element_type=F32)


def _mm_nt(a, b):
    return lax.dot_general(a, b, (((1,), (1,)), ((), ())), preferred_element_type=F32)


def build(S, D, H, E, M, SEG, F, *, G=4, RB=256, SCOPES=False, WAITS=(0, 1, 2, 3, 6, 11, 21), LN_AT=2,
          B1POS=(1, 2), UNROLL=1, name="k7"):
    B1POS = tuple(B1POS)
    NSEG = S // SEG
    L = M + SEG
    scale = float(E) ** -0.5
    NB = S // RB
    HP = H // 2
    HE = H * E
    TS = SEG - M
    P0 = S - NSEG * TS
    RING = 576
    ROFF = RING - P0
    NG = H // G
    NT = D // 128
    TP = SEG

    def scope(n):
        return jax.named_scope(n) if SCOPES else contextlib.nullcontext()

    def kernel(x_hbm, mem0_ref, wq_hbm, wk_hbm, wv_hbm, wo_hbm, w1_hbm, w2_hbm, w3_hbm, w4_hbm,
               out_hbm,
               x_v, hbuf, wk_s, wv_s, wq_s, wo_s, w1_s, w2_s, w3_s, w4_s, sems, wsem, bsem, osem, *rings):
        w_s = (wk_s, wv_s, wq_s)
        ring = [[rings[m * NG + g] for g in range(NG)] for m in range(3)]
        cp_x0 = pltpu.make_async_copy(x_hbm.at[pl.ds(0, P0)], x_v.at[pl.ds(0, P0)], sems.at[0])
        cp_x1 = pltpu.make_async_copy(x_hbm.at[pl.ds(P0, S - P0)], x_v.at[pl.ds(P0, S - P0)], sems.at[1])
        cp_o = [pltpu.make_async_copy(wo_hbm.at[:, pl.ds(j * 128, 128)], wo_s.at[j], sems.at[2 + j])
                for j in range(NT)]
        cp_1 = [pltpu.make_async_copy(w1_hbm.at[:, pl.ds(j * 128, 128)], w1_s.at[j], sems.at[2 + NT + j])
                for j in range(NT)]
        cp_b = [pltpu.make_async_copy(src, dst, bsem.at[i])
                for i, (src, dst) in enumerate(((w2_hbm, w2_s), (w3_hbm, w3_s), (w4_hbm, w4_s)))]
        w_hbm = (wk_hbm, wv_hbm, wq_hbm)
        wo_u = wo_s.bitcast(U32)
        w1_u = w1_s.bitcast(U32)

        def wcat(m, h0, n):
            return jnp.concatenate([pltpu.bitcast(w_s[m][h0 + j], BF16) for j in range(n)], axis=1)

        def phase0(stage):
            src_u = [w.bitcast(U32) for w in w_hbm]
            PPG = G // 2

            def cp_w(m, p):
                return pltpu.make_async_copy(src_u[m].at[:, p, :], stage.at[m, p], wsem.at[m * HP + p])

            def start_w(m, p0, p1):
                def body(p, carry):
                    cp_w(m, p).start()
                    return carry
                lax.fori_loop(p0, p1, body, 0)

            cp_x0.start()
            start_w(0, 0, LN_AT * PPG)
            cp_x1.start()
            start_w(0, LN_AT * PPG, HP)
            start_w(1, 0, HP)
            start_w(2, 0, HP)
            for c in cp_o:
                c.start()

            def ln_rows(r0, n):
                hbuf[pl.ds(r0, n), :] = _ln(x_v[pl.ds(r0, n), :].astype(F32))

            def wait_group(i):
                m, g = divmod(i, NG)
                for p in range(g * PPG, (g + 1) * PPG):
                    cp_w(m, p).wait()

            def bulk(i):
                m, g = divmod(i, NG)
                ws = []
                for p in range(g * PPG, (g + 1) * PPG):
                    a = stage[m, p, pl.ds(0, D // 2, stride=2), :]
                    b = stage[m, p, pl.ds(1, D // 2, stride=2), :]
                    lo = (a & 0xFFFF) | (b << 16)
                    hi = (a >> 16) | (b & np.uint32(0xFFFF0000))
                    w_s[m][2 * p] = lo
                    w_s[m][2 * p + 1] = hi
                    ws += [pltpu.bitcast(lo, BF16), pltpu.bitcast(hi, BF16)]
                ring[m][g][pl.ds(ROFF, P0), :] = _mm(hbuf[pl.ds(0, P0), :], jnp.concatenate(ws, axis=1))

            with scope('start'):
                cp_x0.wait()
                ln_rows(0, P0)
            with scope('bulk'):
                NI = 3 * NG
                for i in range(NI):
                    if i == LN_AT:
                        cp_x1.wait()
                        ln_rows(P0, S - P0)
                    if i in WAITS:
                        hi_ = min([w for w in WAITS if w > i] + [NI])
                        for gg in range(i, hi_):
                            wait_group(gg)
                    bulk(i)
                    if i == NI - 8:
                        for c in cp_1 + cp_b:
                            c.start()

        pl.run_scoped(phase0, pltpu.VMEM((3, HP, D, E), U32))
        with scope('wait_o'):
            for c in cp_o + cp_1:
                c.wait()

        def phase1(t_s, ob):
            def w1_part(part, nparts):
                n = NT // nparts
                return jnp.concatenate([pltpu.bitcast(w1_u[j], BF16) for j in range(part * n, (part + 1) * n)],
                                       axis=1)

            def b1_prep(sp):
                r = pl.ds(pl.multiple_of(sp * SEG, SEG), SEG)
                return _ln(_ln(hbuf[r, :]))

            def b1_mm(hh, sp, part, nparts, clamp=False):
                n = D // nparts
                r = pl.ds(pl.multiple_of(TP + sp * SEG, SEG), SEG)
                t_s[r, pl.ds(part * n, n)] = _gelu(_mm(hh, w1_part(part, nparts)))

            def step(s, mem):
                xs = hbuf[pl.ds(pl.multiple_of(P0 + s * TS, 8), TS), :]
                hs = jnp.concatenate([mem, xs], axis=0)
                rw = pl.ds(pl.multiple_of(lax.rem(s * TS, RING), 8), TS)
                rr = pl.ds(pl.multiple_of(lax.rem(s * SEG + ROFF, RING), SEG), SEG)
                row = lax.broadcasted_iota(jnp.int32, (L, 128), 0)
                col = lax.broadcasted_iota(jnp.int32, (L, 128), 1)
                mask = ((col >= SEG) & (col < L)) | ((col < SEG) & ((row < M) | (col <= row - M)))
                zm = jnp.zeros((16 - M, E), F32)
                zp = jnp.zeros((128 - SEG - 16, E), BF16)

                def proj(m, g):
                    y = _mm(hs, wcat(m, g * G, G))
                    ring[m][g][rw, :] = y[M:, :]
                    return y[:M, :]

                def kv_tile(m, g, j, ymem):
                    tok = ring[m][g][rr, pl.ds(j * E, E)].astype(BF16)
                    mm_ = jnp.concatenate([ymem[:, j * E:(j + 1) * E], zm], axis=0).astype(BF16)
                    return jnp.concatenate([tok, mm_, zp], axis=0)

                def qk(g, qm, km):
                    out = []
                    for j in range(G):
                        q = jnp.concatenate([qm[:, j * E:(j + 1) * E], ring[2][g][rr, pl.ds(j * E, E)]], axis=0)
                        out.append(_mm_nt(q, kv_tile(0, g, j, km)))
                    return out

                def soft(scs):
                    out = []
                    for sc in scs:
                        sc = jnp.where(mask, sc * scale, -1e9)
                        mx = jnp.max(sc, axis=-1, keepdims=True)
                        p = jnp.exp(sc - mx)
                        out.append((p, jnp.sum(p, axis=-1, keepdims=True)))
                    return out

                def pv(g, ps, vm):
                    out = []
                    for j in range(G):
                        out.append(_mm(ps[j][0], kv_tile(1, g, j, vm)) * (1.0 / ps[j][1]))
                    return jnp.concatenate(out, axis=1)

                def oproj(og, g):
                    wo = jnp.concatenate(
                        [pltpu.bitcast(wo_u[j, pl.ds(g * G * E // 2, G * E // 2), :], BF16) for j in range(NT)],
                        axis=1)
                    return _mm(og, wo)

                sp = jnp.maximum(s - 1, 0)
                if B1POS:
                    hh = b1_prep(sp)
                acc = None
                qm, km, vm = proj(2, 0), proj(0, 0), proj(1, 0)
                pend = None
                for g in range(NG):
                    last = g == NG - 1
                    if not last:
                        qm2 = proj(2, g + 1)
                    scs = qk(g, qm, km)
                    if not last:
                        km2 = proj(0, g + 1)
                    elif B1POS == (1, 2):
                        b1_mm(hh, s - 1, 0, 2)
                    elif B1POS == (2,):
                        acc = acc + oproj(*pend)
                    else:
                        acc = acc + oproj(*pend)
                    og = pv(g, soft(scs), vm)
                    if not last:
                        vm2 = proj(1, g + 1)
                    elif B1POS == (1, 2):
                        b1_mm(hh, s - 1, 1, 2)
                    elif B1POS == (2,):
                        b1_mm(hh, s - 1, 0, 1)
                    if g == NG - 2 and B1POS != (1, 2):
                        pend = (og, g)
                    else:
                        y = oproj(og, g)
                        acc = y if acc is None else acc + y
                    if not last:
                        qm, km, vm = qm2, km2, vm2
                r = pl.ds(pl.multiple_of(s * SEG, SEG), SEG)
                hbuf[r, :] = x_v[r, :].astype(F32) + acc[M:, :]
                return acc[:M, :]

            with scope('steps'):
                lax.fori_loop(0, NSEG, step, mem0_ref[...].astype(F32), unroll=UNROLL)

            with scope('wait_b'):
                for c in cp_b:
                    c.wait()
            C = D // 4
            with scope('b1'):
                if B1POS:
                    b1_mm(b1_prep(NSEG - 1), NSEG - 1, 0, 1)
                else:
                    def b1(i, c):
                        r0 = pl.multiple_of(i * RB, RB)
                        hn = _ln(hbuf[pl.ds(r0, RB), :])
                        t_s[pl.ds(r0 + TP, RB), :] = _gelu(_mm(_ln(hn), w1_part(0, 1)))
                        return c
                    lax.fori_loop(0, NB, b1, 0)
                t_s[pl.ds(TP - 8, 8), :] = jnp.zeros((8, D), F32)
                t_s[pl.ds(TP + S, 8), :] = jnp.zeros((8, D), F32)

            def out_copy(i, slot):
                return pltpu.make_async_copy(ob.at[slot], out_hbm.at[pl.ds(pl.multiple_of(i * RB, RB), RB), :],
                                             osem.at[slot])

            def b2(i, c):
                r0 = pl.multiple_of(i * RB, RB)
                h = hbuf[pl.ds(r0, RB), :]
                hn = _ln(h)
                te = t_s[pl.ds(r0 + TP - 8, RB + 16), :]
                n = RB + 16
                g0 = pltpu.roll(te[:, 0 * C:1 * C], 1, 0)
                g1 = pltpu.roll(te[:, 1 * C:2 * C], n - 1, 0)
                g2 = pltpu.roll(te[:, 2 * C:3 * C], 2, 0)
                g3 = pltpu.roll(te[:, 3 * C:4 * C], n - 2, 0)
                gs = jnp.concatenate([g0, g1, g2, g3], axis=1)[8:8 + RB, :]
                x1 = hn + _mm(gs, w2_s[...])
                u = _gelu(_mm(_ln(x1), w3_s[...]))
                res = h + x1 + _mm(u, w4_s[...])
                slot = i % 2

                @pl.when(i >= 2)
                def _():
                    out_copy(i - 2, slot).wait()
                ob[slot] = res.astype(BF16)
                out_copy(i, slot).start()
                return c
            with scope('b2'):
                lax.fori_loop(0, NB, b2, 0)
            with scope('tail'):
                out_copy(NB - 2, 0).wait()
                out_copy(NB - 1, 1).wait()

        pl.run_scoped(phase1, pltpu.VMEM((TP + S + 8, D), F32), pltpu.VMEM((2, RB, D), BF16))

    any_spec = pl.BlockSpec(memory_space=pl.ANY)
    vmem = pl.BlockSpec(memory_space=pltpu.VMEM)
    call = pl.pallas_call(
        kernel,
        out_shape=jax.ShapeDtypeStruct((S, D), BF16),
        in_specs=[any_spec, vmem] + [any_spec] * 8,
        out_specs=any_spec,
        scratch_shapes=[
            pltpu.VMEM((S, D), BF16),
            pltpu.VMEM((S, D), F32),
            pltpu.VMEM((H, D // 2, E), U32),
            pltpu.VMEM((H, D // 2, E), U32),
            pltpu.VMEM((H, D // 2, E), U32),
            pltpu.VMEM((NT, HE, 128), BF16),
            pltpu.VMEM((NT, D, 128), BF16),
            pltpu.VMEM((D, D), BF16),
            pltpu.VMEM((D, F), BF16),
            pltpu.VMEM((F, D), BF16),
            pltpu.SemaphoreType.DMA((2 + 2 * NT,)),
            pltpu.SemaphoreType.DMA((3 * HP,)),
            pltpu.SemaphoreType.DMA((3,)),
            pltpu.SemaphoreType.DMA((2,)),
        ] + [pltpu.VMEM((RING, G * E), F32) for _ in range(3 * NG)],
        compiler_params=pltpu.CompilerParams(vmem_limit_bytes=124 * 2**20),
        name=name,
    )

    def run(A_x, A_mem0, A_Wq, A_Wk, A_Wv, A_Wo, B_w1, B_w2, B_w3, B_w4):
        out = call(A_x.reshape(S, D), A_mem0.reshape(M, D), A_Wq, A_Wk, A_Wv, A_Wo.reshape(H * E, D),
                   B_w1, B_w2, B_w3, B_w4)
        return out.reshape(1, S, D)
    return run


@functools.partial(jax.jit, static_argnames=("A_seg_len",))
def pallas_sequential_preLN__memory_aug_recurrent_mem_tr__mixer_s_mlp__prompt_kernel(
        A_x, A_mem0, A_Wq, A_Wk, A_Wv, A_Wo, A_seg_len, B_x, B_w1, B_w2, B_w3, B_w4):
    del B_x
    _, S, D = A_x.shape
    M = A_mem0.shape[1]
    H, E = A_Wq.shape[1], A_Wq.shape[2]
    F = B_w3.shape[1]
    run = build(S, D, H, E, M, int(A_seg_len), F)
    return run(A_x, A_mem0, A_Wq, A_Wk, A_Wv, A_Wo, B_w1, B_w2, B_w3, B_w4)
```

```python
import contextlib
import functools

import jax
import jax.numpy as jnp
import numpy as np
from jax import lax
from jax.experimental import pallas as pl
from jax.experimental.pallas import tpu as pltpu

F32 = jnp.float32
BF16 = jnp.bfloat16
U32 = jnp.uint32


def _ln(x):
    m = jnp.mean(x, axis=-1, keepdims=True)
    xc = x - m
    v = jnp.mean(xc * xc, axis=-1, keepdims=True)
    return xc * lax.rsqrt(v + 1e-5)


def _gelu(x):
    c = 0.7978845608028654
    return 0.5 * x * (1.0 + jnp.tanh(c * (x + 0.044715 * (x * x * x))))


def _mm(a, b):
    return lax.dot_general(a, b, (((1,), (0,)), ((), ())), preferred_element_type=F32)


def _mm_nt(a, b):
    return lax.dot_general(a, b, (((1,), (1,)), ((), ())), preferred_element_type=F32)


def build(S, D, H, E, M, SEG, F, *, G=4, RB=256, SCOPES=False, WAITS=(0, 1, 2, 3, 6, 11, 21), LNPOS=0, NSUB=2, B2MODE=0, INPLACE=False, BFLHS=True,
          B1POS=(1, 2), UNROLL=2, name="k7"):
    B1POS = tuple(B1POS)
    NSEG = S // SEG
    L = M + SEG
    scale = float(E) ** -0.5
    NB = S // RB
    HP = H // 2
    HE = H * E
    TS = SEG - M
    P0 = S - NSEG * TS
    RING = 576
    ROFF = RING - P0
    NG = H // G
    NT = D // 128
    TP = SEG

    def scope(n):
        return jax.named_scope(n) if SCOPES else contextlib.nullcontext()

    def kernel(x_hbm, mem0_ref, wq_hbm, wk_hbm, wv_hbm, wo_hbm, w1_hbm, w2_hbm, w3_hbm, w4_hbm,
               out_hbm,
               x_v, hbuf, wk_s, wv_s, wq_s, wo_s, w1_s, w2_s, w3_s, w4_s, sems, wsem, bsem, osem, *rings):
        w_s = (wk_s, wv_s, wq_s)
        ring = [[rings[m * NG + g] for g in range(NG)] for m in range(3)]
        cp_x0 = pltpu.make_async_copy(x_hbm.at[pl.ds(0, P0)], x_v.at[pl.ds(0, P0)], sems.at[0])
        cp_x1 = pltpu.make_async_copy(x_hbm.at[pl.ds(P0, S - P0)], x_v.at[pl.ds(P0, S - P0)], sems.at[1])
        cp_o = [pltpu.make_async_copy(wo_hbm.at[:, pl.ds(j * 128, 128)], wo_s.at[j], sems.at[2 + j])
                for j in range(NT)]
        cp_1 = [pltpu.make_async_copy(w1_hbm.at[:, pl.ds(j * 128, 128)], w1_s.at[j], sems.at[2 + NT + j])
                for j in range(NT)]
        cp_b = [pltpu.make_async_copy(src, dst, bsem.at[i])
                for i, (src, dst) in enumerate(((w2_hbm, w2_s), (w3_hbm, w3_s), (w4_hbm, w4_s)))]
        w_hbm = (wk_hbm, wv_hbm, wq_hbm)
        wo_u = wo_s.bitcast(U32)
        w1_u = w1_s.bitcast(U32)

        def wcat(m, h0, n):
            return jnp.concatenate([pltpu.bitcast(w_s[m][h0 + j], BF16) for j in range(n)], axis=1)

        def phase0(stage):
            src_u = [w.bitcast(U32) for w in w_hbm]
            PPG = G // 2

            def cp_w(m, p):
                return pltpu.make_async_copy(src_u[m].at[:, p, :], stage.at[m, p], wsem.at[m * HP + p])

            def start_w(m, p0, p1):
                def body(p, carry):
                    cp_w(m, p).start()
                    return carry
                lax.fori_loop(p0, p1, body, 0)

            cp_x0.start()
            start_w(0, 0, HP)
            start_w(1, 0, HP)
            start_w(2, 0, HP)
            for c in cp_o + [cp_x1] + cp_1:
                c.start()

            def ln_rows(r0, n):
                hbuf[pl.ds(r0, n), :] = _ln(x_v[pl.ds(r0, n), :].astype(F32))

            def wait_group(i):
                m, g = divmod(i, NG)
                for p in range(g * PPG, (g + 1) * PPG):
                    cp_w(m, p).wait()

            def bulk(i):
                m, g = divmod(i, NG)
                ws = []
                for p in range(g * PPG, (g + 1) * PPG):
                    a = stage[m, p, pl.ds(0, D // 2, stride=2), :]
                    b = stage[m, p, pl.ds(1, D // 2, stride=2), :]
                    lo = (a & 0xFFFF) | (b << 16)
                    hi = (a >> 16) | (b & np.uint32(0xFFFF0000))
                    w_s[m][2 * p] = lo
                    w_s[m][2 * p + 1] = hi
                    ws += [pltpu.bitcast(lo, BF16), pltpu.bitcast(hi, BF16)]
                ring[m][g][pl.ds(ROFF, P0), :] = _mm(hbuf[pl.ds(0, P0), :], jnp.concatenate(ws, axis=1))

            with scope('start'):
                cp_x0.wait()
                ln_rows(0, P0)
            with scope('bulk'):
                NI = 3 * NG
                for i in range(NI):
                    if i in WAITS:
                        hi_ = min([w for w in WAITS if w > i] + [NI])
                        for gg in range(i, hi_):
                            wait_group(gg)
                    bulk(i)
                    if i == NI - 8:
                        for c in cp_b:
                            c.start()

        pl.run_scoped(phase0, pltpu.VMEM((3, HP, D, E), U32))
        with scope('wait_o'):
            for c in cp_o + [cp_x1] + cp_1:
                c.wait()

        def phase1(t_s, ob, xs_s):
            def w1_part(part, nparts):
                n = NT // nparts
                return jnp.concatenate([pltpu.bitcast(w1_u[j], BF16) for j in range(part * n, (part + 1) * n)],
                                       axis=1)

            def b1_prep(sp):
                r = pl.ds(pl.multiple_of(sp * SEG, SEG), SEG)
                return _ln(_ln(hbuf[r, :]))

            def b1_mm(hh, sp, part, nparts, clamp=False):
                n = D // nparts
                r = pl.ds(pl.multiple_of(TP + sp * SEG, SEG), SEG)
                t_s[r, pl.ds(part * n, n)] = _gelu(_mm(hh, w1_part(part, nparts)))

            def ln_next(sn):
                r = pl.ds(pl.multiple_of(P0 + jnp.minimum(sn, NSEG - 1) * TS, 8), TS)
                xs_s[lax.rem(sn, 2)] = _ln(x_v[r, :].astype(F32))

            ln_next(0)

            def step(s, mem, bpos):
                xs = xs_s[lax.rem(s, 2)]
                hs = jnp.concatenate([mem, xs], axis=0)
                rw = pl.ds(pl.multiple_of(lax.rem(s * TS, RING), 8), TS)
                rr = pl.ds(pl.multiple_of(lax.rem(s * SEG + ROFF, RING), SEG), SEG)
                row = lax.broadcasted_iota(jnp.int32, (L, 128), 0)
                col = lax.broadcasted_iota(jnp.int32, (L, 128), 1)
                mask = ((col >= SEG) & (col < L)) | ((col < SEG) & ((row < M) | (col <= row - M)))
                zm = jnp.zeros((16 - M, E), F32)
                zp = jnp.zeros((128 - SEG - 16, E), BF16)

                def proj(m, g):
                    y = _mm(hs, wcat(m, g * G, G))
                    ring[m][g][rw, :] = y[M:, :]
                    return y[:M, :]

                def kv_tile(m, g, j, ymem):
                    tok = ring[m][g][rr, pl.ds(j * E, E)].astype(BF16)
                    mm_ = jnp.concatenate([ymem[:, j * E:(j + 1) * E], zm], axis=0).astype(BF16)
                    return jnp.concatenate([tok, mm_, zp], axis=0)

                def qk(g, qm, km):
                    out = []
                    for j in range(G):
                        q = jnp.concatenate([qm[:, j * E:(j + 1) * E], ring[2][g][rr, pl.ds(j * E, E)]], axis=0)
                        out.append(_mm_nt(q, kv_tile(0, g, j, km)))
                    return out

                def soft(scs):
                    out = []
                    for sc in scs:
                        sc = jnp.where(mask, sc * scale, -1e9)
                        mx = jnp.max(sc, axis=-1, keepdims=True)
                        p = jnp.exp(sc - mx)
                        out.append((p, jnp.sum(p, axis=-1, keepdims=True)))
                    return out

                def pv(g, ps, vm):
                    out = []
                    for j in range(G):
                        out.append(_mm(ps[j][0], kv_tile(1, g, j, vm)) * (1.0 / ps[j][1]))
                    return jnp.concatenate(out, axis=1)

                def oproj(og, g):
                    wo = jnp.concatenate(
                        [pltpu.bitcast(wo_u[j, pl.ds(g * G * E // 2, G * E // 2), :], BF16) for j in range(NT)],
                        axis=1)
                    return _mm(og, wo)

                sp = jnp.maximum(s - 1, 0)
                hh = b1_prep(sp)
                ln_next(s + 1)
                acc = None
                qm, km, vm = proj(2, 0), proj(0, 0), proj(1, 0)
                pend = None
                for g in range(NG):
                    last = g == NG - 1
                    if not last:
                        qm2 = proj(2, g + 1)
                    scs = qk(g, qm, km)
                    if not last:
                        km2 = proj(0, g + 1)
                    elif bpos == 0:
                        b1_mm(hh, s - 1, 0, 2)
                    else:
                        acc = acc + oproj(*pend)
                    og = pv(g, soft(scs), vm)
                    if not last:
                        vm2 = proj(1, g + 1)
                    elif bpos == 0:
                        b1_mm(hh, s - 1, 1, 2)
                    else:
                        b1_mm(hh, s - 1, 0, 2)
                    if g == NG - 2 and bpos != 0:
                        pend = (og, g)
                    else:
                        y = oproj(og, g)
                        acc = y if acc is None else acc + y
                    if last and bpos != 0:
                        b1_mm(hh, s - 1, 1, 2)
                    if not last:
                        qm, km, vm = qm2, km2, vm2
                r = pl.ds(pl.multiple_of(s * SEG, SEG), SEG)
                hbuf[r, :] = x_v[r, :].astype(F32) + acc[M:, :]
                return acc[:M, :]

            with scope('steps'):
                def steps(i, mem):
                    for u in range(UNROLL):
                        mem = step(i * UNROLL + u, mem, 1 if u < UNROLL - 1 else 0)
                    return mem
                lax.fori_loop(0, NSEG // UNROLL, steps, mem0_ref[...].astype(F32))

            with scope('wait_b'):
                for c in cp_b:
                    c.wait()
            C = D // 4
            with scope('b1'):
                b1_mm(b1_prep(NSEG - 1), NSEG - 1, 0, 1)
                t_s[pl.ds(TP - 8, 8), :] = jnp.zeros((8, D), F32)
                t_s[pl.ds(TP + S, 8), :] = jnp.zeros((8, D), F32)

            def out_copy(i, slot):
                return pltpu.make_async_copy(ob.at[slot], out_hbm.at[pl.ds(pl.multiple_of(i * RB, RB), RB), :],
                                             osem.at[slot])

            SB = RB // NSUB

            def lhs(v):
                return v.astype(BF16) if BFLHS else v

            def b2(i, c):
                r0 = pl.multiple_of(i * RB, RB)
                slot = i % 2

                def pre(j):
                    r = r0 + j * SB
                    te = t_s[pl.ds(r + TP - 8, SB + 16), :]
                    n = SB + 16
                    g0 = pltpu.roll(te[:, 0 * C:1 * C], 1, 0)
                    g1 = pltpu.roll(te[:, 1 * C:2 * C], n - 1, 0)
                    g2 = pltpu.roll(te[:, 2 * C:3 * C], 2, 0)
                    g3 = pltpu.roll(te[:, 3 * C:4 * C], n - 2, 0)
                    gs = jnp.concatenate([g0, g1, g2, g3], axis=1)[8:8 + SB, :]
                    h = hbuf[pl.ds(r, SB), :]
                    x1 = _ln(h) + _mm(lhs(gs), w2_s[...])
                    if INPLACE:
                        hbuf[pl.ds(r, SB), :] = h + x1
                        return None, lhs(_ln(x1))
                    return h, x1

                def post(j, h, x1):
                    if INPLACE:
                        u = _gelu(_mm(x1, w3_s[...]))
                        res = hbuf[pl.ds(r0 + j * SB, SB), :] + _mm(lhs(u), w4_s[...])
                    else:
                        u = _gelu(_mm(lhs(_ln(x1)), w3_s[...]))
                        res = h + x1 + _mm(lhs(u), w4_s[...])
                    ob[slot, pl.ds(j * SB, SB), :] = res.astype(BF16)

                @pl.when(i >= 2)
                def _():
                    out_copy(i - 2, slot).wait()
                if B2MODE == 0:
                    hx = [pre(j) for j in range(NSUB)]
                    for j in range(NSUB):
                        post(j, *hx[j])
                else:
                    hx = pre(0)
                    for j in range(NSUB):
                        nxt = pre(j + 1) if j + 1 < NSUB else None
                        post(j, *hx)
                        hx = nxt
                out_copy(i, slot).start()
                return c
            with scope('b2'):
                lax.fori_loop(0, NB, b2, 0)
            with scope('tail'):
                out_copy(NB - 2, NB % 2).wait()
                out_copy(NB - 1, (NB + 1) % 2).wait()

        pl.run_scoped(phase1, pltpu.VMEM((TP + S + 8, D), F32), pltpu.VMEM((2, RB, D), BF16), pltpu.VMEM((2, TS, D), F32))

    any_spec = pl.BlockSpec(memory_space=pl.ANY)
    vmem = pl.BlockSpec(memory_space=pltpu.VMEM)
    call = pl.pallas_call(
        kernel,
        out_shape=jax.ShapeDtypeStruct((S, D), BF16),
        in_specs=[any_spec, vmem] + [any_spec] * 8,
        out_specs=any_spec,
        scratch_shapes=[
            pltpu.VMEM((S, D), BF16),
            pltpu.VMEM((S, D), F32),
            pltpu.VMEM((H, D // 2, E), U32),
            pltpu.VMEM((H, D // 2, E), U32),
            pltpu.VMEM((H, D // 2, E), U32),
            pltpu.VMEM((NT, HE, 128), BF16),
            pltpu.VMEM((NT, D, 128), BF16),
            pltpu.VMEM((D, D), BF16),
            pltpu.VMEM((D, F), BF16),
            pltpu.VMEM((F, D), BF16),
            pltpu.SemaphoreType.DMA((2 + 2 * NT,)),
            pltpu.SemaphoreType.DMA((3 * HP,)),
            pltpu.SemaphoreType.DMA((3,)),
            pltpu.SemaphoreType.DMA((2,)),
        ] + [pltpu.VMEM((RING, G * E), F32) for _ in range(3 * NG)],
        compiler_params=pltpu.CompilerParams(vmem_limit_bytes=124 * 2**20),
        name=name,
    )

    def run(A_x, A_mem0, A_Wq, A_Wk, A_Wv, A_Wo, B_w1, B_w2, B_w3, B_w4):
        out = call(A_x.reshape(S, D), A_mem0.reshape(M, D), A_Wq, A_Wk, A_Wv, A_Wo.reshape(H * E, D),
                   B_w1, B_w2, B_w3, B_w4)
        return out.reshape(1, S, D)
    return run


@functools.partial(jax.jit, static_argnames=("A_seg_len",))
def pallas_sequential_preLN__memory_aug_recurrent_mem_tr__mixer_s_mlp__prompt_kernel(
        A_x, A_mem0, A_Wq, A_Wk, A_Wv, A_Wo, A_seg_len, B_x, B_w1, B_w2, B_w3, B_w4):
    del B_x
    _, S, D = A_x.shape
    M = A_mem0.shape[1]
    H, E = A_Wq.shape[1], A_Wq.shape[2]
    F = B_w3.shape[1]
    run = build(S, D, H, E, M, int(A_seg_len), F)
    return run(A_x, A_mem0, A_Wq, A_Wk, A_Wv, A_Wo, B_w1, B_w2, B_w3, B_w4)
```

```python
import functools

import jax
import jax.numpy as jnp
import numpy as np
from jax import lax
from jax.experimental import pallas as pl
from jax.experimental.pallas import tpu as pltpu

F32 = jnp.float32
BF16 = jnp.bfloat16
U32 = jnp.uint32

_LO16 = np.uint32(0x0000FFFF)
_HI16 = np.uint32(0xFFFF0000)

_G = 4
_RB = 256
_NSUB = 2
_UNROLL = 3
_RING = 576
_WAITS = (0, 1, 2, 3, 6, 11, 21)


def _ln(x):
    m = jnp.mean(x, axis=-1, keepdims=True)
    xc = x - m
    v = jnp.mean(xc * xc, axis=-1, keepdims=True)
    return xc * lax.rsqrt(v + 1e-5)


def _gelu(x):
    c = 0.7978845608028654
    return 0.5 * x * (1.0 + jnp.tanh(c * (x + 0.044715 * (x * x * x))))


def _mm(a, b):
    return lax.dot_general(a, b, (((1,), (0,)), ((), ())), preferred_element_type=F32)


def _mm_nt(a, b):
    return lax.dot_general(a, b, (((1,), (1,)), ((), ())), preferred_element_type=F32)


def _build(S, D, H, E, M, SEG, F):
    G, RB, NSUB, UNROLL, RING = _G, _RB, _NSUB, _UNROLL, _RING
    NSEG = S // SEG
    L = M + SEG
    TS = SEG - M
    P0 = S - NSEG * TS
    ROFF = RING - P0
    NG = H // G
    HP = H // 2
    PPG = G // 2
    NT = D // 128
    NB = S // RB
    SB = RB // NSUB
    C = D // 4
    TP = 8
    scale = float(E) ** -0.5
    assert S == NSEG * SEG and E == 128 and M == 8 and SEG == 32 and H % G == 0
    assert RING % SEG == 0 and RING % TS == 0 and ROFF % SEG == 0 and RING >= P0 + TS
    assert P0 % TS == (RING % TS + TS - ROFF % TS) % TS and S % RB == 0 and NB >= 2

    def kernel(x_hbm, mem0_hbm, wq_hbm, wk_hbm, wv_hbm, wo_hbm, w1_hbm, w2_hbm, w3_hbm, w4_hbm,
               out_hbm,
               x_v, mem0_v, hbuf, wk_s, wv_s, wq_s, wo_s, w1_s, w2_s, w3_s, w4_s,
               sems, wsem, bsem, osem, *rings):
        w_hbm = (wk_hbm, wv_hbm, wq_hbm)
        w_s = (wk_s, wv_s, wq_s)
        ring = [[rings[m * NG + g] for g in range(NG)] for m in range(3)]
        wo_u = wo_s.bitcast(U32)
        w1_u = w1_s.bitcast(U32)

        cp_x0 = pltpu.make_async_copy(x_hbm.at[pl.ds(0, P0)], x_v.at[pl.ds(0, P0)], sems.at[0])
        cp_x1 = pltpu.make_async_copy(x_hbm.at[pl.ds(P0, S - P0)], x_v.at[pl.ds(P0, S - P0)],
                                      sems.at[1])
        cp_m = pltpu.make_async_copy(mem0_hbm, mem0_v, sems.at[2])
        cp_o = [pltpu.make_async_copy(wo_hbm.at[:, pl.ds(j * 128, 128)], wo_s.at[j],
                                      sems.at[3 + j]) for j in range(NT)]
        cp_1 = [pltpu.make_async_copy(w1_hbm.at[:, pl.ds(j * 128, 128)], w1_s.at[j],
                                      sems.at[3 + NT + j]) for j in range(NT)]
        cp_b = [pltpu.make_async_copy(src, dst, bsem.at[i])
                for i, (src, dst) in enumerate(((w2_hbm, w2_s), (w3_hbm, w3_s), (w4_hbm, w4_s)))]

        def phase0(stage):
            src_u = [w.bitcast(U32) for w in w_hbm]

            def cp_w(m, p):
                return pltpu.make_async_copy(src_u[m].at[:, p, :], stage.at[m, p],
                                             wsem.at[m * HP + p])

            def start_w(m):
                def body(p, carry):
                    cp_w(m, p).start()
                    return carry
                lax.fori_loop(0, HP, body, 0)

            cp_x0.start()
            for m in range(3):
                start_w(m)
            for c in cp_o + [cp_x1, cp_m] + cp_1:
                c.start()

            cp_x0.wait()
            hbuf[pl.ds(0, P0), :] = _ln(x_v[pl.ds(0, P0), :].astype(F32))

            NI = 3 * NG
            for i in range(NI):
                if i in _WAITS:
                    nxt = min([w for w in _WAITS if w > i] + [NI])
                    for gi in range(i, nxt):
                        m, g = divmod(gi, NG)
                        for p in range(g * PPG, (g + 1) * PPG):
                            cp_w(m, p).wait()
                m, g = divmod(i, NG)
                ws = []
                for p in range(g * PPG, (g + 1) * PPG):
                    even = stage[m, p, pl.ds(0, D // 2, stride=2), :]
                    odd = stage[m, p, pl.ds(1, D // 2, stride=2), :]
                    lo = (even & _LO16) | (odd << 16)
                    hi = (even >> 16) | (odd & _HI16)
                    w_s[m][2 * p] = lo
                    w_s[m][2 * p + 1] = hi
                    ws += [pltpu.bitcast(lo, BF16), pltpu.bitcast(hi, BF16)]
                ring[m][g][pl.ds(ROFF, P0), :] = _mm(hbuf[pl.ds(0, P0), :],
                                                     jnp.concatenate(ws, axis=1))
                if i == NI - NG:
                    for c in cp_b:
                        c.start()

        pl.run_scoped(phase0, pltpu.VMEM((3, HP, D, E), U32))
        for c in cp_o + [cp_x1, cp_m] + cp_1:
            c.wait()

        def phase1(t_s, ob, xs_s):
            def wcat(m, g):
                return jnp.concatenate(
                    [pltpu.bitcast(w_s[m][g * G + j], BF16) for j in range(G)], axis=1)

            def b1_prep(seg):
                r = pl.ds(pl.multiple_of(seg * SEG, SEG), SEG)
                return _ln(_ln(hbuf[r, :]))

            def b1_mm(hh, seg, part, nparts):
                nt = NT // nparts
                w = jnp.concatenate([pltpu.bitcast(w1_u[j], BF16)
                                     for j in range(part * nt, (part + 1) * nt)], axis=1)
                r = pl.ds(pl.multiple_of(TP + seg * SEG, 8), SEG)
                t_s[r, pl.ds(part * nt * 128, nt * 128)] = _gelu(_mm(hh, w))

            def ln_next(sn):
                r = pl.ds(pl.multiple_of(P0 + jnp.minimum(sn, NSEG - 1) * TS, 8), TS)
                xs_s[lax.rem(sn, 2)] = _ln(x_v[r, :].astype(F32))

            def step(s, mem, fill):
                hs = jnp.concatenate([mem, xs_s[lax.rem(s, 2)]], axis=0)
                rw = pl.ds(pl.multiple_of(lax.rem(s * TS, RING), 8), TS)
                rr = pl.ds(pl.multiple_of(lax.rem(s * SEG + ROFF, RING), SEG), SEG)
                row = lax.broadcasted_iota(jnp.int32, (L, 128), 0)
                col = lax.broadcasted_iota(jnp.int32, (L, 128), 1)
                mask = ((col >= SEG) & (col < L)) | (
                    (col < SEG) & ((row < M) | (col <= row - M)))
                zm = jnp.zeros((16 - M, E), F32)
                zp = jnp.zeros((128 - SEG - 16, E), BF16)

                def proj(m, g):
                    y = _mm(hs, wcat(m, g))
                    ring[m][g][rw, :] = y[M:, :]
                    return y[:M, :]

                def kv_tile(m, g, j, y_mem):
                    tok = ring[m][g][rr, pl.ds(j * E, E)].astype(BF16)
                    mk = jnp.concatenate([y_mem[:, j * E:(j + 1) * E], zm], axis=0).astype(BF16)
                    return jnp.concatenate([tok, mk, zp], axis=0)

                def scores(g, qm, km):
                    out = []
                    for j in range(G):
                        q = jnp.concatenate(
                            [qm[:, j * E:(j + 1) * E], ring[2][g][rr, pl.ds(j * E, E)]], axis=0)
                        out.append(_mm_nt(q, kv_tile(0, g, j, km)))
                    return out

                def attend(g, scs, vm):
                    out = []
                    for j, sc in enumerate(scs):
                        sc = jnp.where(mask, sc * scale, -1e9)
                        p = jnp.exp(sc - jnp.max(sc, axis=-1, keepdims=True))
                        l = jnp.sum(p, axis=-1, keepdims=True)
                        out.append(_mm(p, kv_tile(1, g, j, vm)) * (1.0 / l))
                    return jnp.concatenate(out, axis=1)

                def oproj(og, g):
                    k2 = G * E // 2
                    wo = jnp.concatenate([pltpu.bitcast(wo_u[j, pl.ds(g * k2, k2), :], BF16)
                                          for j in range(NT)], axis=1)
                    return _mm(og, wo)

                hh = b1_prep(s - 1) if fill != 2 else None
                ln_next(s + 1)
                acc = None
                pend = None
                qm, km, vm = proj(2, 0), proj(0, 0), proj(1, 0)
                for g in range(NG):
                    last = g == NG - 1
                    if not last:
                        qn = proj(2, g + 1)
                    scs = scores(g, qm, km)
                    if not last:
                        kn = proj(0, g + 1)
                    elif fill == 0:
                        b1_mm(hh, s - 1, 0, 2)
                    else:
                        acc = acc + oproj(*pend)
                    og = attend(g, scs, vm)
                    if not last:
                        vn = proj(1, g + 1)
                    elif fill == 0:
                        b1_mm(hh, s - 1, 1, 2)
                    elif fill == 1:
                        b1_mm(hh, s - 1, 0, 2)
                    if g == NG - 2 and fill != 0:
                        pend = (og, g)
                    else:
                        y = oproj(og, g)
                        acc = y if acc is None else acc + y
                    if last and fill == 1:
                        b1_mm(hh, s - 1, 1, 2)
                    if not last:
                        qm, km, vm = qn, kn, vn
                r = pl.ds(pl.multiple_of(s * SEG, SEG), SEG)
                hbuf[r, :] = x_v[r, :].astype(F32) + acc[M:, :]
                return acc[:M, :]

            ln_next(0)
            assert NSEG % UNROLL == 1
            mem = step(0, mem0_v[...].astype(F32), 2)

            def steps(i, mem):
                for u in range(UNROLL):
                    mem = step(1 + i * UNROLL + u, mem, 1 if u < UNROLL - 1 else 0)
                return mem
            lax.fori_loop(0, NSEG // UNROLL, steps, mem)

            for c in cp_b:
                c.wait()
            b1_mm(b1_prep(NSEG - 1), NSEG - 1, 0, 1)
            t_s[pl.ds(0, TP), :] = jnp.zeros((TP, D), F32)
            t_s[pl.ds(TP + S, 8), :] = jnp.zeros((8, D), F32)

            def out_copy(i, slot, j):
                r = pl.multiple_of(i * RB + j * SB, SB)
                return pltpu.make_async_copy(ob.at[slot, pl.ds(j * SB, SB), :],
                                             out_hbm.at[pl.ds(r, SB), :], osem.at[slot * NSUB + j])

            def mixer(i, carry):
                r0 = pl.multiple_of(i * RB, RB)
                slot = i % 2

                @pl.when(i >= 2)
                def _():
                    for j in range(NSUB):
                        out_copy(i - 2, slot, j).wait()

                hx = []
                for j in range(NSUB):
                    r = r0 + j * SB
                    n = SB + 16
                    te = t_s[pl.ds(r + TP - 8, n), :]
                    gs = jnp.concatenate([
                        pltpu.roll(te[:, 0 * C:1 * C], 1, 0),
                        pltpu.roll(te[:, 1 * C:2 * C], n - 1, 0),
                        pltpu.roll(te[:, 2 * C:3 * C], 2, 0),
                        pltpu.roll(te[:, 3 * C:4 * C], n - 2, 0),
                    ], axis=1)[8:8 + SB, :]
                    h = hbuf[pl.ds(r, SB), :]
                    hx.append((h, _ln(h) + _mm(gs.astype(BF16), w2_s[...])))
                for j, (h, x1) in enumerate(hx):
                    u = _gelu(_mm(_ln(x1).astype(BF16), w3_s[...]))
                    res = h + x1 + _mm(u.astype(BF16), w4_s[...])
                    ob[slot, pl.ds(j * SB, SB), :] = res.astype(BF16)
                    out_copy(i, slot, j).start()
                return carry
            lax.fori_loop(0, NB, mixer, 0)
            for j in range(NSUB):
                out_copy(NB - 2, NB % 2, j).wait()
                out_copy(NB - 1, (NB + 1) % 2, j).wait()

        pl.run_scoped(phase1, pltpu.VMEM((TP + S + 8, D), F32), pltpu.VMEM((2, RB, D), BF16),
                      pltpu.VMEM((2, TS, D), F32))

    any_spec = pl.BlockSpec(memory_space=pl.ANY)
    return pl.pallas_call(
        kernel,
        out_shape=jax.ShapeDtypeStruct((S, D), BF16),
        in_specs=[any_spec] * 10,
        out_specs=any_spec,
        scratch_shapes=[
            pltpu.VMEM((S, D), BF16),
            pltpu.VMEM((M, D), BF16),
            pltpu.VMEM((S, D), F32),
            pltpu.VMEM((H, D // 2, E), U32),
            pltpu.VMEM((H, D // 2, E), U32),
            pltpu.VMEM((H, D // 2, E), U32),
            pltpu.VMEM((NT, H * E, 128), BF16),
            pltpu.VMEM((NT, D, 128), BF16),
            pltpu.VMEM((D, D), BF16),
            pltpu.VMEM((D, F), BF16),
            pltpu.VMEM((F, D), BF16),
            pltpu.SemaphoreType.DMA((3 + 2 * NT,)),
            pltpu.SemaphoreType.DMA((3 * HP,)),
            pltpu.SemaphoreType.DMA((3,)),
            pltpu.SemaphoreType.DMA((2 * NSUB,)),
        ] + [pltpu.VMEM((RING, G * E), F32) for _ in range(3 * NG)],
        compiler_params=pltpu.CompilerParams(vmem_limit_bytes=124 * 2**20),
        name="rmt_mixer_fused",
    )


@functools.partial(jax.jit, static_argnames=("A_seg_len",))
def pallas_sequential_preLN__memory_aug_recurrent_mem_tr__mixer_s_mlp__prompt_kernel(
        A_x, A_mem0, A_Wq, A_Wk, A_Wv, A_Wo, A_seg_len, B_x, B_w1, B_w2, B_w3, B_w4):
    del B_x
    _, S, D = A_x.shape
    M = A_mem0.shape[1]
    H, E = A_Wq.shape[1], A_Wq.shape[2]
    F = B_w3.shape[1]
    call = _build(S, D, H, E, M, int(A_seg_len), F)
    out = call(A_x.reshape(S, D), A_mem0.reshape(M, D), A_Wq, A_Wk, A_Wv, A_Wo.reshape(H * E, D),
               B_w1, B_w2, B_w3, B_w4)
    return out.reshape(1, S, D)
```

```python
import functools

import jax
import jax.numpy as jnp
import numpy as np
from jax import lax
from jax.experimental import pallas as pl
from jax.experimental.pallas import tpu as pltpu

F32 = jnp.float32
BF16 = jnp.bfloat16
U32 = jnp.uint32

_LO16 = np.uint32(0x0000FFFF)
_HI16 = np.uint32(0xFFFF0000)

_G = 4
_RB = 256
_NSUB = 2
_UNROLL = 3
_RING = 576
_WAITS = (0, 1, 2, 3, 6, 11, 21)


def _ln(x):
    m = jnp.mean(x, axis=-1, keepdims=True)
    xc = x - m
    v = jnp.mean(xc * xc, axis=-1, keepdims=True)
    return xc * lax.rsqrt(v + 1e-5)


def _gelu(x):
    c = 0.7978845608028654
    return 0.5 * x * (1.0 + jnp.tanh(c * (x + 0.044715 * (x * x * x))))


def _mm(a, b):
    return lax.dot_general(a, b, (((1,), (0,)), ((), ())), preferred_element_type=F32)


def _mm_nt(a, b):
    return lax.dot_general(a, b, (((1,), (1,)), ((), ())), preferred_element_type=F32)


def _build(S, D, H, E, M, SEG, F):
    G, RB, NSUB, UNROLL, RING = _G, _RB, _NSUB, _UNROLL, _RING
    NSEG = S // SEG
    L = M + SEG
    TS = SEG - M
    P0 = S - NSEG * TS
    ROFF = RING - P0
    NG = H // G
    HP = H // 2
    PPG = G // 2
    NT = D // 128
    NB = S // RB
    SB = RB // NSUB
    C = D // 4
    TP = 8
    scale = float(E) ** -0.5
    assert S == NSEG * SEG and E == 128 and M == 8 and SEG == 32 and H % G == 0
    assert RING % SEG == 0 and RING % TS == 0 and ROFF % SEG == 0 and RING >= P0 + TS
    assert S % RB == 0 and NB >= 2 and P0 % 8 == 0 and NG >= 3 and NSEG % UNROLL == 1

    def kernel(x_hbm, mem0_hbm, wq_hbm, wk_hbm, wv_hbm, wo_hbm, w1_hbm, w2_hbm, w3_hbm, w4_hbm,
               out_hbm,
               x_v, mem0_v, hbuf, wk_s, wv_s, wq_s, wo_s, w1_s, w2_s, w3_s, w4_s,
               sems, wsem, bsem, osem, *rings):
        w_hbm = (wk_hbm, wv_hbm, wq_hbm)
        w_s = (wk_s, wv_s, wq_s)
        ring = [[rings[m * NG + g] for g in range(NG)] for m in range(3)]
        wo_src = wo_hbm.bitcast(U32)
        w1_src = w1_hbm.bitcast(U32)

        cp_x0 = pltpu.make_async_copy(x_hbm.at[pl.ds(0, P0)], x_v.at[pl.ds(0, P0)], sems.at[0])
        cp_x1 = pltpu.make_async_copy(x_hbm.at[pl.ds(P0, S - P0)], x_v.at[pl.ds(P0, S - P0)],
                                      sems.at[1])
        cp_m = pltpu.make_async_copy(mem0_hbm, mem0_v, sems.at[2])
        cp_o = [pltpu.make_async_copy(wo_src.at[:, pl.ds(j * 128, 128)], wo_s.at[j],
                                      sems.at[3 + j]) for j in range(NT)]
        cp_1 = [pltpu.make_async_copy(w1_src.at[:, pl.ds(j * 128, 128)], w1_s.at[j],
                                      sems.at[3 + NT + j]) for j in range(NT)]
        cp_b = [pltpu.make_async_copy(src, dst, bsem.at[i])
                for i, (src, dst) in enumerate(((w2_hbm, w2_s), (w3_hbm, w3_s), (w4_hbm, w4_s)))]

        def phase0(stage):
            src_u = [w.bitcast(U32) for w in w_hbm]

            def cp_w(m, p):
                return pltpu.make_async_copy(src_u[m].at[:, p, :], stage.at[m, p],
                                             wsem.at[m * HP + p])

            def start_w(m):
                def body(p, carry):
                    cp_w(m, p).start()
                    return carry
                lax.fori_loop(0, HP, body, 0)

            cp_x0.start()
            for m in range(3):
                start_w(m)
            for c in cp_o + [cp_x1, cp_m] + cp_1:
                c.start()

            cp_x0.wait()
            hbuf[pl.ds(0, P0), :] = _ln(x_v[pl.ds(0, P0), :].astype(F32))

            NI = 3 * NG
            for i in range(NI):
                if i in _WAITS:
                    nxt = min([w for w in _WAITS if w > i] + [NI])
                    for gi in range(i, nxt):
                        m, g = divmod(gi, NG)
                        for p in range(g * PPG, (g + 1) * PPG):
                            cp_w(m, p).wait()
                m, g = divmod(i, NG)
                ws = []
                for p in range(g * PPG, (g + 1) * PPG):
                    even = stage[m, p, pl.ds(0, D // 2, stride=2), :]
                    odd = stage[m, p, pl.ds(1, D // 2, stride=2), :]
                    lo = (even & _LO16) | (odd << 16)
                    hi = (even >> 16) | (odd & _HI16)
                    w_s[m][2 * p] = lo
                    w_s[m][2 * p + 1] = hi
                    ws += [pltpu.bitcast(lo, BF16), pltpu.bitcast(hi, BF16)]
                ring[m][g][pl.ds(ROFF, P0), :] = _mm(hbuf[pl.ds(0, P0), :],
                                                     jnp.concatenate(ws, axis=1))
                if i == NI - NG:
                    for c in cp_b:
                        c.start()

        pl.run_scoped(phase0, pltpu.VMEM((3, HP, D, E), U32))
        for c in cp_o + [cp_x1, cp_m] + cp_1:
            c.wait()

        def phase1(t_s, ob, xs_s):
            def wcat(m, g):
                return jnp.concatenate(
                    [pltpu.bitcast(w_s[m][g * G + j], BF16) for j in range(G)], axis=1)

            def b1_prep(seg):
                r = pl.ds(pl.multiple_of(seg * SEG, SEG), SEG)
                return _ln(_ln(hbuf[r, :]))

            def b1_mm(hh, seg, part, nparts):
                nt = NT // nparts
                w = jnp.concatenate([pltpu.bitcast(w1_s[j], BF16)
                                     for j in range(part * nt, (part + 1) * nt)], axis=1)
                r = pl.ds(pl.multiple_of(TP + seg * SEG, 8), SEG)
                t_s[r, pl.ds(part * nt * 128, nt * 128)] = _gelu(_mm(hh, w))

            def ln_next(sn):
                r = pl.ds(pl.multiple_of(P0 + jnp.minimum(sn, NSEG - 1) * TS, 8), TS)
                xs_s[lax.rem(sn, 2)] = _ln(x_v[r, :].astype(F32))

            def step(s, mem, fill):
                hs = jnp.concatenate([mem, xs_s[lax.rem(s, 2)]], axis=0)
                rw = pl.ds(pl.multiple_of(lax.rem(s * TS, RING), 8), TS)
                rr = pl.ds(pl.multiple_of(lax.rem(s * SEG + ROFF, RING), SEG), SEG)
                row = lax.broadcasted_iota(jnp.int32, (L, 128), 0)
                col = lax.broadcasted_iota(jnp.int32, (L, 128), 1)
                mask = ((col >= SEG) & (col < L)) | (
                    (col < SEG) & ((row < M) | (col <= row - M)))
                zm = jnp.zeros((16 - M, E), F32)
                zp = jnp.zeros((128 - SEG - 16, E), BF16)

                def proj(m, g):
                    y = _mm(hs, wcat(m, g))
                    ring[m][g][rw, :] = y[M:, :]
                    return y[:M, :]

                def kv_tile(m, g, j, y_mem):
                    tok = ring[m][g][rr, pl.ds(j * E, E)].astype(BF16)
                    mk = jnp.concatenate([y_mem[:, j * E:(j + 1) * E], zm], axis=0).astype(BF16)
                    return jnp.concatenate([tok, mk, zp], axis=0)

                def scores(g, qm, km):
                    out = []
                    for j in range(G):
                        q = jnp.concatenate(
                            [qm[:, j * E:(j + 1) * E], ring[2][g][rr, pl.ds(j * E, E)]], axis=0)
                        out.append(_mm_nt(q, kv_tile(0, g, j, km)))
                    return out

                def attend(g, scs, vm):
                    out = []
                    for j, sc in enumerate(scs):
                        sc = jnp.where(mask, sc * scale, -1e9)
                        p = jnp.exp(sc - jnp.max(sc, axis=-1, keepdims=True))
                        l = jnp.sum(p, axis=-1, keepdims=True)
                        out.append(_mm(p, kv_tile(1, g, j, vm)) * (1.0 / l))
                    return jnp.concatenate(out, axis=1)

                def oproj(og, g):
                    k2 = G * E // 2
                    wo = jnp.concatenate([pltpu.bitcast(wo_s[j, pl.ds(g * k2, k2), :], BF16)
                                          for j in range(NT)], axis=1)
                    return _mm(og, wo)

                hh = b1_prep(s - 1) if fill != 2 else None
                ln_next(s + 1)
                acc = None
                pend = None
                qm, km, vm = proj(2, 0), proj(0, 0), proj(1, 0)
                for g in range(NG):
                    last = g == NG - 1
                    if not last:
                        qn = proj(2, g + 1)
                    scs = scores(g, qm, km)
                    if not last:
                        kn = proj(0, g + 1)
                    elif fill == 0:
                        b1_mm(hh, s - 1, 0, 2)
                    else:
                        acc = acc + oproj(*pend)
                    og = attend(g, scs, vm)
                    if not last:
                        vn = proj(1, g + 1)
                    elif fill == 0:
                        b1_mm(hh, s - 1, 1, 2)
                    elif fill == 1:
                        b1_mm(hh, s - 1, 0, 2)
                    if g == NG - 2 and fill != 0:
                        pend = (og, g)
                    else:
                        y = oproj(og, g)
                        acc = y if acc is None else acc + y
                    if last and fill == 1:
                        b1_mm(hh, s - 1, 1, 2)
                    if not last:
                        qm, km, vm = qn, kn, vn
                r = pl.ds(pl.multiple_of(s * SEG, SEG), SEG)
                hbuf[r, :] = x_v[r, :].astype(F32) + acc[M:, :]
                return acc[:M, :]

            ln_next(0)
            mem = step(0, mem0_v[...].astype(F32), 2)

            def steps(i, mem):
                for u in range(UNROLL):
                    mem = step(1 + i * UNROLL + u, mem, 1 if u < UNROLL - 1 else 0)
                return mem
            lax.fori_loop(0, NSEG // UNROLL, steps, mem)

            for c in cp_b:
                c.wait()
            b1_mm(b1_prep(NSEG - 1), NSEG - 1, 0, 1)
            t_s[pl.ds(0, TP), :] = jnp.zeros((TP, D), F32)
            t_s[pl.ds(TP + S, 8), :] = jnp.zeros((8, D), F32)

            def out_copy(i, slot, j):
                r = pl.multiple_of(i * RB + j * SB, SB)
                return pltpu.make_async_copy(ob.at[slot, pl.ds(j * SB, SB), :],
                                             out_hbm.at[pl.ds(r, SB), :], osem.at[slot * NSUB + j])

            def mixer(i, carry):
                r0 = pl.multiple_of(i * RB, RB)
                slot = i % 2

                @pl.when(i >= 2)
                def _():
                    for j in range(NSUB):
                        out_copy(i - 2, slot, j).wait()

                hx = []
                for j in range(NSUB):
                    r = r0 + j * SB
                    n = SB + 16
                    te = t_s[pl.ds(r + TP - 8, n), :]
                    gs = jnp.concatenate([
                        pltpu.roll(te[:, 0 * C:1 * C], 1, 0),
                        pltpu.roll(te[:, 1 * C:2 * C], n - 1, 0),
                        pltpu.roll(te[:, 2 * C:3 * C], 2, 0),
                        pltpu.roll(te[:, 3 * C:4 * C], n - 2, 0),
                    ], axis=1)[8:8 + SB, :]
                    h = hbuf[pl.ds(r, SB), :]
                    hx.append((h, _ln(h) + _mm(gs.astype(BF16), w2_s[...])))
                for j, (h, x1) in enumerate(hx):
                    u = _gelu(_mm(_ln(x1).astype(BF16), w3_s[...]))
                    res = h + x1 + _mm(u.astype(BF16), w4_s[...])
                    ob[slot, pl.ds(j * SB, SB), :] = res.astype(BF16)
                    out_copy(i, slot, j).start()
                return carry
            lax.fori_loop(0, NB, mixer, 0)
            for j in range(NSUB):
                out_copy(NB - 2, NB % 2, j).wait()
                out_copy(NB - 1, (NB + 1) % 2, j).wait()

        pl.run_scoped(phase1, pltpu.VMEM((TP + S + 8, D), F32), pltpu.VMEM((2, RB, D), BF16),
                      pltpu.VMEM((2, TS, D), F32))

    any_spec = pl.BlockSpec(memory_space=pl.ANY)
    return pl.pallas_call(
        kernel,
        out_shape=jax.ShapeDtypeStruct((S, D), BF16),
        in_specs=[any_spec] * 10,
        out_specs=any_spec,
        scratch_shapes=[
            pltpu.VMEM((S, D), BF16),
            pltpu.VMEM((M, D), BF16),
            pltpu.VMEM((S, D), F32),
            pltpu.VMEM((H, D // 2, E), U32),
            pltpu.VMEM((H, D // 2, E), U32),
            pltpu.VMEM((H, D // 2, E), U32),
            pltpu.VMEM((NT, H * E // 2, 128), U32),
            pltpu.VMEM((NT, D // 2, 128), U32),
            pltpu.VMEM((D, D), BF16),
            pltpu.VMEM((D, F), BF16),
            pltpu.VMEM((F, D), BF16),
            pltpu.SemaphoreType.DMA((3 + 2 * NT,)),
            pltpu.SemaphoreType.DMA((3 * HP,)),
            pltpu.SemaphoreType.DMA((3,)),
            pltpu.SemaphoreType.DMA((2 * NSUB,)),
        ] + [pltpu.VMEM((RING, G * E), F32) for _ in range(3 * NG)],
        compiler_params=pltpu.CompilerParams(vmem_limit_bytes=124 * 2**20),
        name="rmt_mixer_fused",
    )


@functools.partial(jax.jit, static_argnames=("A_seg_len",))
def pallas_sequential_preLN__memory_aug_recurrent_mem_tr__mixer_s_mlp__prompt_kernel(
        A_x, A_mem0, A_Wq, A_Wk, A_Wv, A_Wo, A_seg_len, B_x, B_w1, B_w2, B_w3, B_w4):
    del B_x
    _, S, D = A_x.shape
    M = A_mem0.shape[1]
    H, E = A_Wq.shape[1], A_Wq.shape[2]
    F = B_w3.shape[1]
    call = _build(S, D, H, E, M, int(A_seg_len), F)
    out = call(A_x.reshape(S, D), A_mem0.reshape(M, D), A_Wq, A_Wk, A_Wv, A_Wo.reshape(H * E, D),
               B_w1, B_w2, B_w3, B_w4)
    return out.reshape(1, S, D)
```

```python
import functools

import jax
import jax.numpy as jnp
import numpy as np
from jax import lax
from jax.experimental import pallas as pl
from jax.experimental.pallas import tpu as pltpu

F32 = jnp.float32
BF16 = jnp.bfloat16
U32 = jnp.uint32

_LO16 = np.uint32(0x0000FFFF)
_HI16 = np.uint32(0xFFFF0000)

_G = 4
_RB = 256
_NSUB = 2
_UNROLL = 3
_RING = 576
_WAITS = (0, 1, 2, 3, 6, 11, 21)


def _ln(x):
    m = jnp.mean(x, axis=-1, keepdims=True)
    xc = x - m
    v = jnp.mean(xc * xc, axis=-1, keepdims=True)
    return xc * lax.rsqrt(v + 1e-5)


def _gelu(x):
    c = 0.7978845608028654
    return 0.5 * x * (1.0 + jnp.tanh(c * (x + 0.044715 * (x * x * x))))


def _mm(a, b):
    return lax.dot_general(a, b, (((1,), (0,)), ((), ())), preferred_element_type=F32)


def _mm_nt(a, b):
    return lax.dot_general(a, b, (((1,), (1,)), ((), ())), preferred_element_type=F32)


def _build(S, D, H, E, M, SEG, F):
    G, RB, NSUB, UNROLL, RING = _G, _RB, _NSUB, _UNROLL, _RING
    NSEG = S // SEG
    L = M + SEG
    TS = SEG - M
    P0 = S - NSEG * TS
    ROFF = RING - P0
    NG = H // G
    HP = H // 2
    PPG = G // 2
    NT = D // 128
    NB = S // RB
    SB = RB // NSUB
    C = D // 4
    TP = 8
    scale = float(E) ** -0.5
    assert S == NSEG * SEG and E == 128 and M == 8 and SEG == 32 and H % G == 0
    assert RING % SEG == 0 and RING % TS == 0 and ROFF % SEG == 0 and RING >= P0 + TS
    assert S % RB == 0 and NB >= 2 and P0 % 8 == 0 and NG >= 3 and NSEG % UNROLL == 1

    def kernel(x_hbm, mem0_hbm, wq_hbm, wk_hbm, wv_hbm, wo_hbm, w1_hbm, w2_hbm, w3_hbm, w4_hbm,
               out_hbm,
               x_v, mem0_v, hbuf, wk_s, wv_s, wq_s, wo_s, w1_s, w2_s, w3_s, w4_s,
               sems, wsem, osem, *rings):
        w_hbm = (wk_hbm, wv_hbm, wq_hbm)
        w_s = (wk_s, wv_s, wq_s)
        ring = [[rings[m * NG + g] for g in range(NG)] for m in range(3)]
        wo_src = wo_hbm.bitcast(U32)
        w1_src = w1_hbm.bitcast(U32)

        cp_x0 = pltpu.make_async_copy(x_hbm.at[pl.ds(0, P0)], x_v.at[pl.ds(0, P0)], sems.at[0])
        cp_a = [pltpu.make_async_copy(wo_src.at[:, pl.ds(j * 128, 128)], wo_s.at[j], sems.at[1])
                for j in range(NT)]
        cp_a += [pltpu.make_async_copy(x_hbm.at[pl.ds(P0, S - P0)], x_v.at[pl.ds(P0, S - P0)],
                                       sems.at[1]),
                 pltpu.make_async_copy(mem0_hbm, mem0_v, sems.at[1])]
        cp_a += [pltpu.make_async_copy(w1_src.at[:, pl.ds(j * 128, 128)], w1_s.at[j], sems.at[1])
                 for j in range(NT)]
        cp_b = [pltpu.make_async_copy(src, dst, sems.at[2])
                for src, dst in ((w2_hbm, w2_s), (w3_hbm, w3_s), (w4_hbm, w4_s))]

        def phase0(stage):
            src_u = [w.bitcast(U32) for w in w_hbm]

            NI = 3 * NG
            bounds = [w for w in _WAITS if w < NI] + [NI]

            def cp_w(m, p, k):
                return pltpu.make_async_copy(src_u[m].at[:, p, :], stage.at[m, p], wsem.at[k])

            cp_x0.start()
            for m in range(3):
                for k in range(len(bounds) - 1):
                    lo, hi = max(bounds[k], m * NG), min(bounds[k + 1], (m + 1) * NG)
                    if lo < hi:
                        def body(p, carry, m=m, k=k):
                            cp_w(m, p, k).start()
                            return carry
                        lax.fori_loop((lo - m * NG) * PPG, (hi - m * NG) * PPG, body, 0)
            for c in cp_a:
                c.start()

            cp_x0.wait()
            hbuf[pl.ds(0, P0), :] = _ln(x_v[pl.ds(0, P0), :].astype(F32))

            for i in range(NI):
                if i in bounds:
                    k = bounds.index(i)
                    for gi in range(i, bounds[k + 1]):
                        m, g = divmod(gi, NG)
                        for p in range(g * PPG, (g + 1) * PPG):
                            cp_w(m, p, k).wait()
                m, g = divmod(i, NG)
                ws = []
                for p in range(g * PPG, (g + 1) * PPG):
                    even = stage[m, p, pl.ds(0, D // 2, stride=2), :]
                    odd = stage[m, p, pl.ds(1, D // 2, stride=2), :]
                    lo = (even & _LO16) | (odd << 16)
                    hi = (even >> 16) | (odd & _HI16)
                    w_s[m][2 * p] = lo
                    w_s[m][2 * p + 1] = hi
                    ws += [pltpu.bitcast(lo, BF16), pltpu.bitcast(hi, BF16)]
                ring[m][g][pl.ds(ROFF, P0), :] = _mm(hbuf[pl.ds(0, P0), :],
                                                     jnp.concatenate(ws, axis=1))
                if i == NI - NG:
                    for c in cp_b:
                        c.start()

        pl.run_scoped(phase0, pltpu.VMEM((3, HP, D, E), U32))
        for c in cp_a:
            c.wait()

        def phase1(t_s, ob, xs_s):
            def wcat(m, g):
                return jnp.concatenate(
                    [pltpu.bitcast(w_s[m][g * G + j], BF16) for j in range(G)], axis=1)

            def b1_prep(seg):
                r = pl.ds(pl.multiple_of(seg * SEG, SEG), SEG)
                return _ln(_ln(hbuf[r, :]))

            def b1_mm(hh, seg, part, nparts):
                nt = NT // nparts
                w = jnp.concatenate([pltpu.bitcast(w1_s[j], BF16)
                                     for j in range(part * nt, (part + 1) * nt)], axis=1)
                r = pl.ds(pl.multiple_of(TP + seg * SEG, 8), SEG)
                t_s[r, pl.ds(part * nt * 128, nt * 128)] = _gelu(_mm(hh, w))

            def ln_next(sn):
                r = pl.ds(pl.multiple_of(P0 + jnp.minimum(sn, NSEG - 1) * TS, 8), TS)
                xs_s[lax.rem(sn, 2)] = _ln(x_v[r, :].astype(F32))

            def step(s, mem, fill):
                hs = jnp.concatenate([mem, xs_s[lax.rem(s, 2)]], axis=0)
                rw = pl.ds(pl.multiple_of(lax.rem(s * TS, RING), 8), TS)
                rr = pl.ds(pl.multiple_of(lax.rem(s * SEG + ROFF, RING), SEG), SEG)
                row = lax.broadcasted_iota(jnp.int32, (L, 128), 0)
                col = lax.broadcasted_iota(jnp.int32, (L, 128), 1)
                mask = ((col >= SEG) & (col < L)) | (
                    (col < SEG) & ((row < M) | (col <= row - M)))
                zm = jnp.zeros((16 - M, E), F32)
                zp = jnp.zeros((128 - SEG - 16, E), BF16)

                def proj(m, g):
                    y = _mm(hs, wcat(m, g))
                    ring[m][g][rw, :] = y[M:, :]
                    return y[:M, :]

                def kv_tile(m, g, j, y_mem):
                    tok = ring[m][g][rr, pl.ds(j * E, E)].astype(BF16)
                    mk = jnp.concatenate([y_mem[:, j * E:(j + 1) * E], zm], axis=0).astype(BF16)
                    return jnp.concatenate([tok, mk, zp], axis=0)

                def scores(g, qm, km):
                    out = []
                    for j in range(G):
                        q = jnp.concatenate(
                            [qm[:, j * E:(j + 1) * E], ring[2][g][rr, pl.ds(j * E, E)]], axis=0)
                        out.append(_mm_nt(q, kv_tile(0, g, j, km)))
                    return out

                def attend(g, scs, vm):
                    out = []
                    for j, sc in enumerate(scs):
                        sc = jnp.where(mask, sc * scale, -1e9)
                        p = jnp.exp(sc - jnp.max(sc, axis=-1, keepdims=True))
                        l = jnp.sum(p, axis=-1, keepdims=True)
                        out.append(_mm(p, kv_tile(1, g, j, vm)) * (1.0 / l))
                    return jnp.concatenate(out, axis=1)

                def oproj(og, g):
                    k2 = G * E // 2
                    wo = jnp.concatenate([pltpu.bitcast(wo_s[j, pl.ds(g * k2, k2), :], BF16)
                                          for j in range(NT)], axis=1)
                    return _mm(og, wo)

                hh = b1_prep(s - 1) if fill != 2 else None
                ln_next(s + 1)
                acc = None
                pend = None
                qm, km, vm = proj(2, 0), proj(0, 0), proj(1, 0)
                for g in range(NG):
                    last = g == NG - 1
                    if not last:
                        qn = proj(2, g + 1)
                    scs = scores(g, qm, km)
                    if not last:
                        kn = proj(0, g + 1)
                    elif fill == 0:
                        b1_mm(hh, s - 1, 0, 2)
                    else:
                        acc = acc + oproj(*pend)
                    og = attend(g, scs, vm)
                    if not last:
                        vn = proj(1, g + 1)
                    elif fill == 0:
                        b1_mm(hh, s - 1, 1, 2)
                    elif fill == 1:
                        b1_mm(hh, s - 1, 0, 2)
                    if g == NG - 2 and fill != 0:
                        pend = (og, g)
                    else:
                        y = oproj(og, g)
                        acc = y if acc is None else acc + y
                    if last and fill == 1:
                        b1_mm(hh, s - 1, 1, 2)
                    if not last:
                        qm, km, vm = qn, kn, vn
                r = pl.ds(pl.multiple_of(s * SEG, SEG), SEG)
                hbuf[r, :] = x_v[r, :].astype(F32) + acc[M:, :]
                return acc[:M, :]

            ln_next(0)
            mem = step(0, mem0_v[...].astype(F32), 2)

            def steps(i, mem):
                for u in range(UNROLL):
                    mem = step(1 + i * UNROLL + u, mem, 1 if u < UNROLL - 1 else 0)
                return mem
            lax.fori_loop(0, NSEG // UNROLL, steps, mem)

            for c in cp_b:
                c.wait()
            b1_mm(b1_prep(NSEG - 1), NSEG - 1, 0, 1)
            t_s[pl.ds(0, TP), :] = jnp.zeros((TP, D), F32)
            t_s[pl.ds(TP + S, 8), :] = jnp.zeros((8, D), F32)

            def out_copy(i, slot, j):
                r = pl.multiple_of(i * RB + j * SB, SB)
                return pltpu.make_async_copy(ob.at[slot, pl.ds(j * SB, SB), :],
                                             out_hbm.at[pl.ds(r, SB), :], osem.at[slot * NSUB + j])

            def mixer(i, carry):
                r0 = pl.multiple_of(i * RB, RB)
                slot = i % 2

                @pl.when(i >= 2)
                def _():
                    for j in range(NSUB):
                        out_copy(i - 2, slot, j).wait()

                hx = []
                for j in range(NSUB):
                    r = r0 + j * SB
                    n = SB + 16
                    te = t_s[pl.ds(r + TP - 8, n), :]
                    gs = jnp.concatenate([
                        pltpu.roll(te[:, 0 * C:1 * C], 1, 0),
                        pltpu.roll(te[:, 1 * C:2 * C], n - 1, 0),
                        pltpu.roll(te[:, 2 * C:3 * C], 2, 0),
                        pltpu.roll(te[:, 3 * C:4 * C], n - 2, 0),
                    ], axis=1)[8:8 + SB, :]
                    h = hbuf[pl.ds(r, SB), :]
                    hx.append((h, _ln(h) + _mm(gs.astype(BF16), w2_s[...])))
                for j, (h, x1) in enumerate(hx):
                    u = _gelu(_mm(_ln(x1).astype(BF16), w3_s[...]))
                    res = h + x1 + _mm(u.astype(BF16), w4_s[...])
                    ob[slot, pl.ds(j * SB, SB), :] = res.astype(BF16)
                    out_copy(i, slot, j).start()
                return carry
            lax.fori_loop(0, NB, mixer, 0)
            for j in range(NSUB):
                out_copy(NB - 2, NB % 2, j).wait()
                out_copy(NB - 1, (NB + 1) % 2, j).wait()

        pl.run_scoped(phase1, pltpu.VMEM((TP + S + 8, D), F32), pltpu.VMEM((2, RB, D), BF16),
                      pltpu.VMEM((2, TS, D), F32))

    any_spec = pl.BlockSpec(memory_space=pl.ANY)
    return pl.pallas_call(
        kernel,
        out_shape=jax.ShapeDtypeStruct((S, D), BF16),
        in_specs=[any_spec] * 10,
        out_specs=any_spec,
        scratch_shapes=[
            pltpu.VMEM((S, D), BF16),
            pltpu.VMEM((M, D), BF16),
            pltpu.VMEM((S, D), F32),
            pltpu.VMEM((H, D // 2, E), U32),
            pltpu.VMEM((H, D // 2, E), U32),
            pltpu.VMEM((H, D // 2, E), U32),
            pltpu.VMEM((NT, H * E // 2, 128), U32),
            pltpu.VMEM((NT, D // 2, 128), U32),
            pltpu.VMEM((D, D), BF16),
            pltpu.VMEM((D, F), BF16),
            pltpu.VMEM((F, D), BF16),
            pltpu.SemaphoreType.DMA((3,)),
            pltpu.SemaphoreType.DMA((len(_WAITS),)),
            pltpu.SemaphoreType.DMA((2 * NSUB,)),
        ] + [pltpu.VMEM((RING, G * E), F32) for _ in range(3 * NG)],
        compiler_params=pltpu.CompilerParams(vmem_limit_bytes=124 * 2**20),
        name="rmt_mixer_fused",
    )


@functools.partial(jax.jit, static_argnames=("A_seg_len",))
def pallas_sequential_preLN__memory_aug_recurrent_mem_tr__mixer_s_mlp__prompt_kernel(
        A_x, A_mem0, A_Wq, A_Wk, A_Wv, A_Wo, A_seg_len, B_x, B_w1, B_w2, B_w3, B_w4):
    del B_x
    _, S, D = A_x.shape
    M = A_mem0.shape[1]
    H, E = A_Wq.shape[1], A_Wq.shape[2]
    F = B_w3.shape[1]
    call = _build(S, D, H, E, M, int(A_seg_len), F)
    out = call(A_x.reshape(S, D), A_mem0.reshape(M, D), A_Wq, A_Wk, A_Wv, A_Wo.reshape(H * E, D),
               B_w1, B_w2, B_w3, B_w4)
    return out.reshape(1, S, D)
```
